```python
import jax
import jax.numpy as jnp

def _softmax(x, axis=-1):
    return jax.nn.softmax(x, axis=axis)
def _gelu(x):
    return jax.nn.gelu(x, approximate=True)
def _silu(x):
    return jax.nn.silu(x)
def _sigmoid(x):
    return jax.nn.sigmoid(x)
def _layernorm(x, axis=-1, eps=1e-5):
    m = jnp.mean(x, axis=axis, keepdims=True)
    v = jnp.var(x, axis=axis, keepdims=True)
    return (x - m) / jnp.sqrt(v + eps)
def _scatter_add(tgt, idx, src, axis=0):
    return tgt.at[idx].add(src)
def _segment_sum(src, seg, n):
    return jax.ops.segment_sum(src, seg, n)
class _Rng:
    def __init__(self, key):
        self._k = key
    def _next(self):
        self._k, sub = jax.random.split(self._k)
        return sub
    def normal(self, shape):
        return jax.random.normal(self._next(), shape, dtype=jnp.bfloat16)
    def randint(self, lo, hi, shape):
        return jax.random.randint(self._next(), shape, lo, hi, dtype=jnp.int32)
    def uniform(self, shape, lo=0.0, hi=1.0):
        return jax.random.uniform(self._next(), shape, jnp.bfloat16, lo, hi)
    def permutation(self, n):
        return jax.random.permutation(self._next(), n)


kernel_name = 'interleave_layers__softmax_full_mha__ssm_conv_h3__prompt'

def setup_inputs():
    _rng = _Rng(jax.random.key(int.from_bytes(__import__("os").urandom(4), "little")))
    _w = (lambda a: (lambda t: t.astype(jnp.bfloat16) if jnp.issubdtype(t.dtype, jnp.floating) else t)(jnp.asarray(a)))
    def _A_setup():
        B, S, D = 1, 2048, 1024
        return {
            "x": _w((lambda *s: _rng.normal(s) * 0.05)(B, S, D)),
            "wqkv": _w((lambda *s: _rng.normal(s) * 0.05)(D, 3 * D)),
            "wo": _w((lambda *s: _rng.normal(s) * 0.05)(D, D)),
        }
    _A_in = _A_setup()

    def _B_setup():
        B, S, D = 1, 2048, 1024
        ks = 4
        return {
            "q": _w((lambda *s: _rng.normal(s) * 0.05)(B, S, D)),
            "k": _w((lambda *s: _rng.normal(s) * 0.05)(B, S, D)),
            "v": _w((lambda *s: _rng.normal(s) * 0.05)(B, S, D)),
            "shift_k": _w((lambda *s: _rng.normal(s) * 0.05)(D, ks) * 0.5),
            "ssm_k": _w((lambda *s: _rng.normal(s) * 0.05)(D, S) * (1.0 / S ** 0.5)),
            "ssm_D": _w((lambda *s: _rng.normal(s) * 0.05)(D)),
        }
    _B_in = _B_setup()

    return {
        "A_x": _A_in["x"],
        "A_wqkv": _A_in["wqkv"],
        "A_wo": _A_in["wo"],
        "B_q": _B_in["q"],
        "B_k": _B_in["k"],
        "B_v": _B_in["v"],
        "B_shift_k": _B_in["shift_k"],
        "B_ssm_k": _B_in["ssm_k"],
        "B_ssm_D": _B_in["ssm_D"],
    }

def reference(A_x, A_wqkv, A_wo, B_q, B_k, B_v, B_shift_k, B_ssm_k, B_ssm_D):
    def _A_ref(x, wqkv, wo):
        B, S, D = x.shape
        H = 32; Dh = D // H
        qkv = (lambda x, *d: x.transpose(*d))((x @ wqkv).reshape(B, S, 3, H, Dh), 2, 0, 3, 1, 4)
        q, k, v = qkv[0], qkv[1], qkv[2]
        scale = Dh ** -0.5
        scores = jnp.einsum("bhqd,bhkd->bhqk", q, k) * scale
        p = _softmax(scores, axis=-1)
        o = jnp.einsum("bhqk,bhkd->bhqd", p, v)
        return (lambda x, *d: x.transpose(*d))(o, 0, 2, 1, 3).reshape(B, S, D) @ wo

    def _B_ref(q, k, v, shift_k, ssm_k, ssm_D):
        B, S, D = q.shape
        ks = shift_k.shape[-1]
        k_pad = jnp.pad(k, ((0, 0), (ks - 1, 0), (0, 0)))
        k_shift = jnp.zeros_like(k)
        for t in range(ks):
            k_shift = k_shift + k_pad[:, t:t + S, :] * shift_k[:, ks - 1 - t][None, None, :]
        kv = k_shift * v
        L = 2 * S
        kv_pad = jnp.pad(kv, ((0, 0), (0, S), (0, 0)))
        kf_pad = jnp.pad(ssm_k, ((0, 0), (0, S)))
        kv_f = (lambda x, axes=(-2,-1): jnp.fft.rfft2(x.astype(jnp.float32), axes=axes))(kv_pad[:, None, :, :], axes=(1, 2))
        kf_f = (lambda x, axes=(-2,-1): jnp.fft.rfft2(x.astype(jnp.float32), axes=axes))(kf_pad[:, None, :], axes=(1, 2))
        kf_f = (lambda x, *d: x.transpose(*d))(kf_f, 1, 2, 0)
        y_f = kv_f * kf_f[None, :, :, :]
        y = (lambda x, s, axes=(-2,-1): jnp.fft.irfft2(x, s=s, axes=axes).astype(jnp.bfloat16))(y_f, (1, L), axes=(1, 2))[:, 0, :S, :]
        y = y + kv * ssm_D[None, None, :]
        return q * y

    x = A_x
    x = x + _A_ref(_layernorm(x, axis=-1), A_wqkv, A_wo)
    x = x + _B_ref(_layernorm(x, axis=-1), B_k, B_v, B_shift_k, B_ssm_k, B_ssm_D)
    x = x + _A_ref(_layernorm(x, axis=-1), A_wqkv, A_wo)
    x = x + _B_ref(_layernorm(x, axis=-1), B_k, B_v, B_shift_k, B_ssm_k, B_ssm_D)
    return x
```

```python
import numpy as np
import jax
import jax.numpy as jnp
import jax.experimental.pallas as pl
import jax.experimental.pallas.tpu as pltpu

S, D, H, DH = 2048, 1024, 32, 32
C = 128
NC = S // C
DT = 512
TQ = 512
CH = 512
RT = 256
F32, BF16 = jnp.float32, jnp.bfloat16

_th = np.pi * np.outer(np.arange(C) + 0.5, np.arange(2 * C)) / C
_FWD = np.concatenate([np.cos(_th), -np.sin(_th)], 0).astype(np.float32)
_INV = (_FWD[:, C:].T / C).astype(np.float32)


def _dot(a, b):
    return jnp.dot(a, b, preferred_element_type=F32)


def _dot_t(a, b):
    return jax.lax.dot_general(a, b, (((1,), (1,)), ((), ())), preferred_element_type=F32)


def _ln(x):
    d = x - jnp.mean(x, -1, keepdims=True)
    return d * jax.lax.rsqrt(jnp.mean(d * d, -1, keepdims=True) + 1e-5)


def _kernel(x_h, wqkv_h, wo_h, k_h, v_h, h_h, sk_ref, sd_ref, fwd_ref, inv_ref, out_ref,
            xin, wqkv, wo, kin, vin, hin, sems, x_s, wT, k_s, qT, vT, oT, s_ref, m_ref,
            y_s, kp, X, W):
    cps = [pltpu.make_async_copy(a, b, sems.at[i]) for i, (a, b) in enumerate(
        [(wqkv_h, wqkv), (x_h, xin), (wo_h, wo), (k_h, kin), (v_h, vin), (h_h, hin)])]
    for c in cps:
        c.start()

    def project(r0, xn):
        xn = xn.astype(BF16)
        k_s[pl.ds(r0, RT), :] = _dot(xn, wqkv[:, D:2 * D]).astype(BF16)
        qT[:, pl.ds(r0, RT)] = (_dot_t(wT[0:D, :], xn) * (DH ** -0.5 * np.log2(np.e))).astype(BF16)
        vT[:, pl.ds(r0, RT)] = _dot_t(wT[D:2 * D, :], xn).astype(BF16)

    NQ = S // TQ
    U = H * NQ

    def idx(i):
        return i // NQ, pl.multiple_of((i % NQ) * TQ, TQ)

    def qk(i, slot):
        h, q0 = idx(i)
        g = pl.multiple_of((h // 4) * 128, 128)
        q = qT[pl.ds(g, 128), pl.ds(q0, TQ)]
        r = jax.lax.broadcasted_iota(jnp.int32, (128, TQ), 0)
        q = jnp.where((r // DH) == (h % 4), q, jnp.zeros_like(q))
        m = None
        for c in range(S // CH):
            s = _dot(k_s[c * CH:(c + 1) * CH, pl.ds(g, 128)], q)
            s_ref[slot, c * CH:(c + 1) * CH, :] = s
            mc = jnp.max(s.reshape(CH // 8, 8, TQ), 0)
            m = mc if m is None else jnp.maximum(m, mc)
        m_ref[slot] = jnp.broadcast_to(jnp.max(m, 0, keepdims=True), (8, TQ))

    def pv(i, slot):
        h, q0 = idx(i)
        g = pl.multiple_of(h * DH, DH)
        m = m_ref[slot]
        l = o = None
        for c in range(S // CH):
            s = s_ref[slot, c * CH:(c + 1) * CH, :].reshape(CH // 8, 8, TQ)
            p = jnp.exp2(s - m[None])
            lc = jnp.sum(p, 0)
            oc = _dot(vT[pl.ds(g, DH), c * CH:(c + 1) * CH], p.reshape(CH, TQ).astype(BF16))
            l = lc if l is None else l + lc
            o = oc if o is None else o + oc
        oT[pl.ds(g, DH), pl.ds(q0, TQ)] = (o / jnp.sum(l, 0, keepdims=True)).astype(BF16)

    def attention():
        qk(0, 0)

        def body(j, c):
            qk(2 * j + 1, 1)
            pv(2 * j, 0)
            qk(jnp.minimum(2 * j + 2, U - 1), 0)
            pv(2 * j + 1, 1)
            return c
        jax.lax.fori_loop(0, U // 2, body, 0)

    def conv(t, c):
        cols = pl.ds(pl.multiple_of(t * DT, DT), DT)
        kp[0:8, :] = jnp.zeros((8, DT), F32)
        kp[8:, :] = kin[:, cols].astype(F32)
        sk = sk_ref[:, cols].astype(F32)
        sd = sd_ref[:, cols].astype(F32)
        for j in range(NC):
            ks = kp[8 + j * C:8 + (j + 1) * C, :] * sk[0:1]
            for a in range(1, 4):
                ks = ks + kp[8 - a + j * C:8 - a + (j + 1) * C, :] * sk[a:a + 1]
            kv = ks * vin[j * C:(j + 1) * C, cols].astype(F32)
            y_s[j * C:(j + 1) * C, cols] = kv * sd
            X[j] = _dot(fwd_ref[:, 0:C], kv.astype(BF16))
            if j == 0:
                W[0] = _dot_t(fwd_ref[:, C:], hin[cols, 0:C])
            else:
                W[j] = _dot_t(fwd_ref[...], hin[cols, (j - 1) * C:(j + 1) * C])

        def mac(i, c2):
            re = pl.ds(pl.multiple_of((i // (DT // 128)) * 8, 8), 8)
            im = pl.ds(pl.multiple_of((i // (DT // 128)) * 8 + C, 8), 8)
            ln = pl.ds(pl.multiple_of((i % (DT // 128)) * 128, 128), 128)
            for n in reversed(range(NC)):
                ar = ai = None
                for j in range(n + 1):
                    xr, xi = X[j, re, ln], X[j, im, ln]
                    wr, wi = W[n - j, re, ln], W[n - j, im, ln]
                    pr, pi = xr * wr - xi * wi, xr * wi + xi * wr
                    ar = pr if ar is None else ar + pr
                    ai = pi if ai is None else ai + pi
                X[n, re, ln] = ar
                X[n, im, ln] = ai
            return c2
        jax.lax.fori_loop(0, (C // 8) * (DT // 128), mac, 0)
        for j in range(NC):
            y = _dot(inv_ref[...], X[j].astype(BF16))
            y_s[j * C:(j + 1) * C, cols] += y.astype(BF16).astype(F32)
        return c

    def post(r0):
        rows = pl.ds(r0, RT)
        x = x_s[rows, :] + _dot(oT[:, rows].T, wo[...])
        return x + _ln(x) * y_s[rows, :]

    cps[0].wait()
    for j in range(D // 256):
        wT[j * 256:(j + 1) * 256, :] = wqkv[:, j * 256:(j + 1) * 256].T
        wT[D + j * 256:D + (j + 1) * 256, :] = wqkv[:, 2 * D + j * 256:2 * D + (j + 1) * 256].T
    cps[1].wait()

    def p1(i, c):
        r0 = pl.multiple_of(i * RT, RT)
        x = xin[pl.ds(r0, RT), :].astype(F32)
        x_s[pl.ds(r0, RT), :] = x
        project(r0, _ln(x))
        return c
    jax.lax.fori_loop(0, S // RT, p1, 0)
    attention()
    for c in cps[2:]:
        c.wait()
    jax.lax.fori_loop(0, D // DT, conv, 0)

    def p2(i, c):
        r0 = pl.multiple_of(i * RT, RT)
        x = post(r0)
        x_s[pl.ds(r0, RT), :] = x
        project(r0, _ln(x))
        return c
    jax.lax.fori_loop(0, S // RT, p2, 0)
    attention()

    def p3(i, c):
        r0 = pl.multiple_of(i * RT, RT)
        out_ref[pl.ds(r0, RT), :] = post(r0).astype(BF16)
        return c
    jax.lax.fori_loop(0, S // RT, p3, 0)


@jax.jit
def pallas_interleave_layers__softmax_full_mha__ssm_conv_h3__prompt_kernel(
        A_x, A_wqkv, A_wo, B_q, B_k, B_v, B_shift_k, B_ssm_k, B_ssm_D):
    hbm = pl.BlockSpec(memory_space=pl.ANY)
    vm = pl.BlockSpec(memory_space=pltpu.VMEM)
    V = pltpu.VMEM
    out = pl.pallas_call(
        _kernel,
        out_shape=jax.ShapeDtypeStruct((S, D), BF16),
        in_specs=[hbm] * 6 + [vm] * 4,
        out_specs=vm,
        scratch_shapes=[
            V((S, D), BF16), V((D, 3 * D), BF16), V((D, D), BF16), V((S, D), BF16),
            V((S, D), BF16), V((D, S), BF16), pltpu.SemaphoreType.DMA((6,)),
            V((S, D), F32), V((2 * D, D), BF16), V((S, D), BF16), V((D, S), BF16),
            V((D, S), BF16), V((D, S), BF16), V((2, S, TQ), F32), V((2, 8, TQ), F32),
            V((S, D), F32), V((S + 8, DT), F32), V((NC, 2 * C, DT), F32), V((NC, 2 * C, DT), F32),
        ],
        compiler_params=pltpu.CompilerParams(vmem_limit_bytes=120 << 20),
    )(A_x.reshape(S, D), A_wqkv, A_wo, B_k.reshape(S, D), B_v.reshape(S, D), B_ssm_k,
      B_shift_k.T, B_ssm_D.reshape(1, D), jnp.asarray(_FWD, BF16), jnp.asarray(_INV, BF16))
    return out.reshape(1, S, D)
```

```python
import numpy as np
import jax
import jax.numpy as jnp
import jax.experimental.pallas as pl
import jax.experimental.pallas.tpu as pltpu

S, D, H, DH = 2048, 1024, 32, 32
C = 128
NC = S // C
DT = 512
TQ = 512
CH = 512
RT = 256
F32, BF16 = jnp.float32, jnp.bfloat16

_th = np.pi * np.outer(np.arange(C) + 0.5, np.arange(2 * C)) / C
_FWD = np.concatenate([np.cos(_th), -np.sin(_th)], 0).astype(np.float32)
_INV = (_FWD[:, C:].T / C).astype(np.float32)


def _dot(a, b):
    return jnp.dot(a, b, preferred_element_type=F32)


def _dot_t(a, b):
    return jax.lax.dot_general(a, b, (((1,), (1,)), ((), ())), preferred_element_type=F32)


def _ln(x):
    d = x - jnp.mean(x, -1, keepdims=True)
    return d * jax.lax.rsqrt(jnp.mean(d * d, -1, keepdims=True) + 1e-5)


def _kernel(x_h, wqkv_h, wo_h, k_h, v_h, h_h, sk_ref, sd_ref, fwd_ref, inv_ref, out_ref,
            xin, wqkv, wo, kin, vin, hin, sems, x_s, wT, k_s, qT, vT, oT, s_ref, m_ref,
            y_s, kp, X, W):
    cps = [pltpu.make_async_copy(a, b, sems.at[i]) for i, (a, b) in enumerate(
        [(wqkv_h, wqkv), (x_h, xin), (wo_h, wo), (k_h, kin), (v_h, vin), (h_h, hin)])]
    for c in cps:
        c.start()

    def project(r0, xn):
        xn = xn.astype(BF16)
        k_s[pl.ds(r0, RT), :] = _dot(xn, wqkv[:, D:2 * D]).astype(BF16)
        qT[:, pl.ds(r0, RT)] = (_dot_t(wT[0:D, :], xn) * (DH ** -0.5 * np.log2(np.e))).astype(BF16)
        vT[:, pl.ds(r0, RT)] = _dot_t(wT[D:2 * D, :], xn).astype(BF16)

    NQ = S // TQ
    U = H * NQ

    def idx(i):
        return i // NQ, pl.multiple_of((i % NQ) * TQ, TQ)

    def qk(i, slot):
        h, q0 = idx(i)
        g = pl.multiple_of((h // 4) * 128, 128)
        q = qT[pl.ds(g, 128), pl.ds(q0, TQ)]
        r = jax.lax.broadcasted_iota(jnp.int32, (128, TQ), 0)
        q = jnp.where((r // DH) == (h % 4), q, jnp.zeros_like(q))
        m = None
        for c in range(S // CH):
            s = _dot(k_s[c * CH:(c + 1) * CH, pl.ds(g, 128)], q)
            s_ref[slot, c * CH:(c + 1) * CH, :] = s
            mc = jnp.max(s.reshape(CH // 8, 8, TQ), 0)
            m = mc if m is None else jnp.maximum(m, mc)
        m_ref[slot] = jnp.broadcast_to(jnp.max(m, 0, keepdims=True), (8, TQ))

    def pv(i, slot):
        h, q0 = idx(i)
        g = pl.multiple_of(h * DH, DH)
        m = m_ref[slot]
        l = o = None
        for c in range(S // CH):
            s = s_ref[slot, c * CH:(c + 1) * CH, :].reshape(CH // 8, 8, TQ)
            p = jnp.exp2(s - m[None])
            lc = jnp.sum(p, 0)
            oc = _dot(vT[pl.ds(g, DH), c * CH:(c + 1) * CH], p.reshape(CH, TQ).astype(BF16))
            l = lc if l is None else l + lc
            o = oc if o is None else o + oc
        oT[pl.ds(g, DH), pl.ds(q0, TQ)] = (o / jnp.sum(l, 0, keepdims=True)).astype(BF16)

    def attention(with_mac):
        qk(0, 0)

        def body(j, c):
            qk(2 * j + 1, 1)
            pv(2 * j, 0)
            if with_mac:
                mac(2 * j)
                mac(2 * j + 1)
            qk(jnp.minimum(2 * j + 2, U - 1), 0)
            pv(2 * j + 1, 1)
            return c
        jax.lax.fori_loop(0, U // 2, body, 0)

    def conv(t, c):
        cols = pl.ds(pl.multiple_of(t * DT, DT), DT)
        kp[0:8, :] = jnp.zeros((8, DT), F32)
        kp[8:, :] = kin[:, cols].astype(F32)
        sk = sk_ref[:, cols].astype(F32)
        sd = sd_ref[:, cols].astype(F32)
        for j in range(NC):
            ks = kp[8 + j * C:8 + (j + 1) * C, :] * sk[0:1]
            for a in range(1, 4):
                ks = ks + kp[8 - a + j * C:8 - a + (j + 1) * C, :] * sk[a:a + 1]
            kv = ks * vin[j * C:(j + 1) * C, cols].astype(F32)
            y_s[j * C:(j + 1) * C, cols] = kv * sd
            X[j, :, cols] = _dot(fwd_ref[:, 0:C], kv.astype(BF16))
            if j == 0:
                W[0, :, cols] = _dot_t(fwd_ref[:, C:], hin[cols, 0:C])
            else:
                W[j, :, cols] = _dot_t(fwd_ref[...], hin[cols, (j - 1) * C:(j + 1) * C])

        return c

    def mac(i):
        re = pl.ds(pl.multiple_of((i // 8) * 8, 8), 8)
        im = pl.ds(pl.multiple_of((i // 8) * 8 + C, 8), 8)
        ln = pl.ds(pl.multiple_of((i % 8) * 128, 128), 128)
        for n in reversed(range(NC)):
            ar = ai = None
            for j in range(n + 1):
                xr, xi = X[j, re, ln], X[j, im, ln]
                wr, wi = W[n - j, re, ln], W[n - j, im, ln]
                pr, pi = xr * wr - xi * wi, xr * wi + xi * wr
                ar = pr if ar is None else ar + pr
                ai = pi if ai is None else ai + pi
            X[n, re, ln] = ar
            X[n, im, ln] = ai

    def conv_inv(j, c):
        rows = pl.ds(pl.multiple_of(j * C, C), C)
        y = _dot(inv_ref[...], X[j].astype(BF16))
        y_s[rows, :] += y.astype(BF16).astype(F32)
        return c

    def post(r0):
        rows = pl.ds(r0, RT)
        x = x_s[rows, :] + _dot(oT[:, rows].T, wo[...])
        return x + _ln(x) * y_s[rows, :]

    cps[0].wait()
    for j in range(D // 256):
        wT[j * 256:(j + 1) * 256, :] = wqkv[:, j * 256:(j + 1) * 256].T
        wT[D + j * 256:D + (j + 1) * 256, :] = wqkv[:, 2 * D + j * 256:2 * D + (j + 1) * 256].T
    cps[1].wait()

    def p1(i, c):
        r0 = pl.multiple_of(i * RT, RT)
        x = xin[pl.ds(r0, RT), :].astype(F32)
        x_s[pl.ds(r0, RT), :] = x
        project(r0, _ln(x))
        return c
    jax.lax.fori_loop(0, S // RT, p1, 0)
    for c in cps[2:]:
        c.wait()
    jax.lax.fori_loop(0, D // DT, conv, 0)
    attention(True)
    jax.lax.fori_loop(0, NC, conv_inv, 0)

    def p2(i, c):
        r0 = pl.multiple_of(i * RT, RT)
        x = post(r0)
        x_s[pl.ds(r0, RT), :] = x
        project(r0, _ln(x))
        return c
    jax.lax.fori_loop(0, S // RT, p2, 0)
    attention(False)

    def p3(i, c):
        r0 = pl.multiple_of(i * RT, RT)
        xin[pl.ds(r0, RT), :] = post(r0).astype(BF16)
        out_cp(i).start()
        return c

    def out_cp(i):
        rows = pl.ds(pl.multiple_of(i * RT, RT), RT)
        return pltpu.make_async_copy(xin.at[rows], out_ref.at[rows], sems.at[6])
    jax.lax.fori_loop(0, S // RT, p3, 0)
    for i in range(S // RT):
        out_cp(i).wait()


@jax.jit
def pallas_interleave_layers__softmax_full_mha__ssm_conv_h3__prompt_kernel(
        A_x, A_wqkv, A_wo, B_q, B_k, B_v, B_shift_k, B_ssm_k, B_ssm_D):
    hbm = pl.BlockSpec(memory_space=pl.ANY)
    vm = pl.BlockSpec(memory_space=pltpu.VMEM)
    V = pltpu.VMEM
    out = pl.pallas_call(
        _kernel,
        out_shape=jax.ShapeDtypeStruct((S, D), BF16),
        in_specs=[hbm] * 6 + [vm] * 4,
        out_specs=hbm,
        scratch_shapes=[
            V((S, D), BF16), V((D, 3 * D), BF16), V((D, D), BF16), V((S, D), BF16),
            V((S, D), BF16), V((D, S), BF16), pltpu.SemaphoreType.DMA((7,)),
            V((S, D), F32), V((2 * D, D), BF16), V((S, D), BF16), V((D, S), BF16),
            V((D, S), BF16), V((D, S), BF16), V((2, S, TQ), F32), V((2, 8, TQ), F32),
            V((S, D), F32), V((S + 8, DT), F32), V((NC, 2 * C, D), F32), V((NC, 2 * C, D), F32),
        ],
        compiler_params=pltpu.CompilerParams(vmem_limit_bytes=120 << 20),
    )(A_x.reshape(S, D), A_wqkv, A_wo, B_k.reshape(S, D), B_v.reshape(S, D), B_ssm_k,
      B_shift_k.T, B_ssm_D.reshape(1, D), jnp.asarray(_FWD, BF16), jnp.asarray(_INV, BF16))
    return out.reshape(1, S, D)
```
